```python
import os as _os
_os.environ.setdefault('JAX_PLATFORMS', 'cpu')
import jax
import jax.numpy as jnp

def _softmax(x, axis=-1):
    return jax.nn.softmax(x, axis=axis)

def _gelu(x):
    return jax.nn.gelu(x, approximate=True)

def _silu(x):
    return jax.nn.silu(x)

def _sigmoid(x):
    return jax.nn.sigmoid(x)

def _layernorm(x, axis=-1, eps=1e-05):
    m = jnp.mean(x, axis=axis, keepdims=True)
    v = jnp.var(x, axis=axis, keepdims=True)
    return (x - m) / jnp.sqrt(v + eps)

def _scatter_add(tgt, idx, src, axis=0):
    return tgt.at[idx].add(src)

def _segment_sum(src, seg, n):
    return jax.ops.segment_sum(src, seg, n)

class _Rng:

    def __init__(self, key):
        self._k = key

    def _next(self):
        self._k, sub = jax.random.split(self._k)
        return sub

    def normal(self, shape):
        return jax.random.normal(self._next(), shape, dtype=jnp.bfloat16)

    def randint(self, lo, hi, shape):
        return jax.random.randint(self._next(), shape, lo, hi, dtype=jnp.int32)

    def uniform(self, shape, lo=0.0, hi=1.0):
        return jax.random.uniform(self._next(), shape, jnp.bfloat16, lo, hi)

    def permutation(self, n):
        return jax.random.permutation(self._next(), n)
kernel_name = 'standalone__window_attn_twins__vision'

def setup_inputs():
    _rng = _Rng(jax.random.key(int.from_bytes(__import__("os").urandom(4), "little")))
    _w = lambda a: (lambda t: t.astype(jnp.bfloat16) if jnp.issubdtype(t.dtype, jnp.floating) else t)(jnp.asarray(a))
    H = W = 384 // 8 * 8
    C = 96
    return {'x': _w((lambda *s: _rng.normal(s) * 0.4)(1, H, W, C)), 'wq': _w((lambda *s: _rng.normal(s) * 0.4)(C, C)), 'wkv': _w((lambda *s: _rng.normal(s) * 0.4)(C, 2 * C)), 'wo': _w((lambda *s: _rng.normal(s) * 0.05)(C, C))}

def reference(x, wq, wkv, wo):
    B, H, W, C = x.shape
    win = 8
    nh, nw = (H // win, W // win)
    xs = x.reshape(B, nh, win, nw, win, C).mean(axis=(2, 4)).reshape(B, nh * nw, C)
    q = x.reshape(B, H * W, C) @ wq
    kv = xs @ wkv
    k, v = (kv[..., :C].copy(), kv[..., C:].copy())
    scale = C ** (-0.5)
    p = _softmax(jnp.einsum('bqc,bkc->bqk', q, k) * scale, axis=-1)
    o = jnp.einsum('bqk,bkc->bqc', p, v) @ wo
    return o.reshape(B, H, W, C)
```

```python
import functools
import numpy as np
import jax
import jax.numpy as jnp
from jax import lax
import jax.experimental.pallas as pl
import jax.experimental.pallas.tpu as pltpu

WIN = 8
LOG2E = 1.4426950408889634
NT = (((1,), (1,)), ((), ()))


def make(G=4, KT=128, U=3, order='ab', flags=None, pack=True):
    f32, bf16, u32 = jnp.float32, jnp.bfloat16, jnp.uint32

    def kernel(x_hbm, wq_ref, wkv_ref, wo_ref, o_hbm, xbuf, xs_ref, k_ref, vt_ref, s_ref, m_ref, obuf, in_sems, out_sems):
        H, C, W = xbuf.shape
        NH, NW = H // WIN, W // WIN
        NK = NH * NW
        WT = W // 128
        HB = G * U // WT
        assert HB * WT == G * U
        NIT = H // HB

        def in_copy(i):
            return pltpu.make_async_copy(x_hbm.at[pl.ds(i * WIN, WIN)], xbuf.at[pl.ds(i * WIN, WIN)], in_sems.at[i])

        def start(i, c):
            in_copy(i).start()
            return c
        lax.fori_loop(0, NH, start, 0)

        r = lax.broadcasted_iota(jnp.int32, (NW, W), 0)
        c = lax.broadcasted_iota(jnp.int32, (NW, W), 1)
        pm = jnp.where((c // WIN) == r, 1.0 / (WIN * WIN), 0.0).astype(bf16)

        def pool(i, carry):
            in_copy(i).wait()
            acc = xbuf[i * WIN].astype(f32)
            for a in range(1, WIN):
                acc = acc + xbuf[i * WIN + a].astype(f32)
            hi = acc.astype(bf16)
            lo = (acc - hi.astype(f32)).astype(bf16)
            xs = lax.dot_general(pm, hi, NT, preferred_element_type=f32) + lax.dot_general(pm, lo, NT, preferred_element_type=f32)
            xs_ref[pl.ds(pl.multiple_of(i * NW, NW), NW), :] = xs.astype(bf16)
            return carry
        lax.fori_loop(0, NH, pool, 0)

        xs = xs_ref[...]
        kv = jnp.dot(xs, wkv_ref[...], preferred_element_type=f32).astype(bf16)
        k = kv[:, :C]
        v = kv[:, C:]
        kp = lax.dot_general(k, wq_ref[...], NT, preferred_element_type=f32) * (C ** -0.5 * LOG2E)
        wot = wo_ref[...].astype(f32).T.astype(bf16)
        vt = lax.dot_general(wot, v, NT, preferred_element_type=f32).astype(bf16)
        if pack:
            k_ref[...] = pltpu.bitcast(kp.astype(bf16), u32)
            vt_ref[...] = pltpu.bitcast(vt, u32)
        else:
            k_ref[...] = kp.astype(bf16)
            vt_ref[...] = vt

        def load_k(r0, n):
            if pack:
                return pltpu.bitcast(k_ref[r0 // 2:(r0 + n) // 2, :], bf16)
            return k_ref[r0:r0 + n, :]

        def load_vt(r0, n):
            if pack:
                return pltpu.bitcast(vt_ref[:, r0:r0 + n], bf16)
            return vt_ref[:, r0:r0 + n]

        def tiles(u):
            return [divmod(u * G + g, WT) for g in range(G)]

        def load_x(h0, u):
            return jnp.concatenate([xbuf[h0 + a, :, t * 128:(t + 1) * 128] for a, t in tiles(u)], axis=1)

        def step(xt, m_cur, store):
            m_new = None
            acc = None
            l = None
            for r0 in range(0, NK, KT):
                if m_cur is not None:
                    s_cur = s_ref[r0:r0 + KT, :]
                def do_a():
                    nonlocal m_new
                    s = jnp.dot(load_k(r0, KT), xt, preferred_element_type=f32)
                    s_ref[r0:r0 + KT, :] = s
                    mm = jnp.max(s.reshape(KT // 8, 8, G * 128), axis=0)
                    m_new = mm if m_new is None else jnp.maximum(m_new, mm)
                def do_b():
                    nonlocal acc, l
                    p = jnp.exp2(s_cur.reshape(KT // 8, 8, G * 128) - m_cur[None])
                    ll = jnp.sum(p, axis=0)
                    l = ll if l is None else l + ll
                    o = jnp.dot(load_vt(r0, KT), p.reshape(KT, G * 128).astype(bf16), preferred_element_type=f32)
                    acc = o if acc is None else acc + o
                for ch in order:
                    if ch == 'a' and xt is not None: do_a()
                    if ch == 'b' and m_cur is not None: do_b()
            if m_cur is not None:
                inv = 1.0 / jnp.sum(l, axis=0, keepdims=True)
                store((acc * inv).astype(bf16))
            if xt is not None:
                return jnp.broadcast_to(jnp.max(m_new, axis=0, keepdims=True), m_new.shape)

        def out_copy(i, slot):
            return pltpu.make_async_copy(obuf.at[slot], o_hbm.at[pl.ds(i * HB, HB)], out_sems.at[slot])

        m_ref[...] = step(load_x(0, 0), None, None)

        def body(i, carry):
            slot = i % 2

            @pl.when(i >= 2)
            def _():
                out_copy(i - 2, slot).wait()

            m = m_ref[...]
            for u in range(U):
                def store(o, u=u):
                    for g, (a, t) in enumerate(tiles(u)):
                        obuf[slot, a, :, t * 128:(t + 1) * 128] = o[:, g * 128:(g + 1) * 128]
                if u + 1 < U:
                    xt = load_x(i * HB, u + 1)
                else:
                    xt = load_x(jnp.minimum(i + 1, NIT - 1) * HB, 0)
                m = step(xt, m, store)
            m_ref[...] = m
            out_copy(i, slot).start()
            return carry
        lax.fori_loop(0, NIT, body, 0)
        out_copy(NIT - 2, 0).wait()
        out_copy(NIT - 1, 1).wait()

    def f(x, wq, wkv, wo):
        B, H, W, C = x.shape
        xt = jnp.transpose(x, (0, 1, 3, 2)).reshape(H, C, W)
        NK = (H // WIN) * (W // WIN)
        HB = G * U // (W // 128)
        ot = pl.pallas_call(
            kernel,
            out_shape=jax.ShapeDtypeStruct((H, C, W), x.dtype),
            in_specs=[pl.BlockSpec(memory_space=pl.ANY), pl.BlockSpec(memory_space=pltpu.VMEM), pl.BlockSpec(memory_space=pltpu.VMEM), pl.BlockSpec(memory_space=pltpu.VMEM)],
            out_specs=pl.BlockSpec(memory_space=pl.ANY),
            scratch_shapes=[
                pltpu.VMEM((H, C, W), jnp.bfloat16),
                pltpu.VMEM((NK, C), jnp.bfloat16),
                pltpu.VMEM((NK // 2, C), u32) if pack else pltpu.VMEM((NK, C), jnp.bfloat16),
                pltpu.VMEM((C // 2, NK), u32) if pack else pltpu.VMEM((C, NK), jnp.bfloat16),
                pltpu.VMEM((NK, G * 128), f32),
                pltpu.VMEM((8, G * 128), f32),
                pltpu.VMEM((2, HB, C, W), jnp.bfloat16),
                pltpu.SemaphoreType.DMA((H // WIN,)),
                pltpu.SemaphoreType.DMA((2,)),
            ],
            compiler_params=pltpu.CompilerParams(vmem_limit_bytes=100 * 1024 * 1024, flags=flags),
        )(xt, wq, wkv, wo)
        return jnp.transpose(ot.reshape(B, H, C, W), (0, 1, 3, 2))
    return f


@jax.jit
def pallas_standalone__window_attn_twins__vision_kernel(x, wq, wkv, wo):
    return make(G=3,KT=128,U=1)(x, wq, wkv, wo)
```

```python
import functools

import jax
import jax.numpy as jnp
from jax import lax
import jax.experimental.pallas as pl
import jax.experimental.pallas.tpu as pltpu

WIN = 8
LANES = 128
UNIT = 48
N = 6
BLOCKS = 6
EARLY_KEYS = 144
CHUNK = 4
RING = 3
LEAD, TAIL = 2, 2
LATE = (0, 1)
LOG2E = 1.4426950408889634
NT = (((1,), (1,)), ((), ()))

_T = (-1.25, -0.75, -0.25, 0.25, 0.75, 1.25)
_PRODUCTS = [('D', j) for j in range(N)] + [('E', j) for j in range(N)] + [
    pr for i in range(N) for j in range(i + 1, N) for pr in (('X', i, j), ('X', j, i), ('Z', i, j))]

_ORDER = (
    'X10|X01 Z01|X02 X30|X20 Z02|X03 Z03|X40 X05|X04 Z04|E0,X50 Z05,D0 X13|X12|X21 Z12|X31 Z13|X14 X15,X41 Z14|X51 Z15,E1,D1|X23,X32 Z23|X24 X25|X42 Z24|E2,Z25 X52,D2|X34 X35|X43 Z34|X53 Z35,E3,D3|X45|E4,X54 Z45,D4,E5,D5',
)
_SPARE = (23, 26)


def _cells(pr):
    if pr[0] == 'D':
        return [(i, pr[1]) for i in range(N)]
    if pr[0] == 'E':
        return [(pr[1], j) for j in range(N)]
    if pr[0] == 'X':
        return [(pr[1], pr[2])]
    return [(pr[2], pr[1]), (pr[1], pr[2])]


def _schedule(groups):
    work = [[(u, g, (k[0],) + tuple(map(int, k[1:]))) for k in rnd.split()]
            for u in range(BLOCKS) for phase in _ORDER[u % len(_ORDER)].split('|')
            for g in range(groups) for rnd in phase.split(',')]
    scores = [(u, j, r) for u in range(BLOCKS) for j in range(N)
              for r in range(EARLY_KEYS, N * groups * LANES, UNIT)]
    n_spare = (len(scores) - sum(4 - len(w) for w in work)) // 4 - LEAD - TAIL
    per_block = len(work) // BLOCKS
    spare = [u * per_block + e for e in _SPARE for u in range(BLOCKS)][:n_spare]
    rounds = [[]] * LEAD
    for n, w in enumerate(work):
        rounds = rounds + [w] + [[]] * spare.count(n)
    rounds = rounds + [[]] * (n_spare - len(spare) + TAIL)

    first = {}
    for n, rnd in enumerate(rounds):
        for u, g, pr in rnd:
            for i, j in _cells(pr):
                first.setdefault((u, i * groups + g, j), n)

    def free(u, j, r):
        return max(first[u, r // LANES, j], first[u, (r + UNIT - 1) // LANES, j])

    span = groups * LANES
    last = [s for s in scores if s[:2] == LATE][-4 * TAIL:]
    todo = sorted((s for s in scores if s not in last),
                  key=lambda s: (free(s[0], s[1], s[2] // span * span), s))
    jobs = []
    for n, rnd in enumerate(rounds):
        jobs += [('value',) + w for w in rnd]
        for _ in range(4 - len(rnd)):
            if not todo:
                todo, last = last, []
            s = next((s for s in todo if free(*s) <= n), todo[-1])
            todo.remove(s)
            jobs.append(('score',) + s)
    return jobs + [('score',) + s for s in todo + last]


def _tree_sum(xs):
    xs = list(xs)
    while len(xs) > 1:
        xs = [xs[i] + xs[i + 1] if i + 1 < len(xs) else xs[i] for i in range(0, len(xs), 2)]
    return xs[0]


def _fold(s):
    s = s.reshape(-1, 2, 8, LANES)
    halves = [s[:, 0].reshape(-1, LANES), s[:, 1].reshape(-1, LANES)]
    return jnp.concatenate(halves, axis=1).astype(jnp.bfloat16)


def _unfold(b):
    b = b.astype(jnp.float32)
    return jnp.concatenate(
        [b[r:r + 8, c:c + LANES] for r in range(0, b.shape[0], 8) for c in (0, LANES)], axis=0)


def _slab_max(s):
    return jnp.max(s.reshape(-1, 8, LANES), axis=0)


def _slab_sum(s):
    return jnp.sum(s.reshape(-1, 8, LANES), axis=0)


def _shift(maxes):
    m = functools.reduce(jnp.maximum, maxes)
    m = jnp.broadcast_to(jnp.max(m, axis=0, keepdims=True), m.shape)
    return m + jnp.log2(jnp.sum(_tree_sum(jnp.exp2(v - m) for v in maxes), axis=0, keepdims=True))


def _pack(a):
    return pltpu.bitcast(a.astype(jnp.bfloat16), jnp.uint32)


def _unpack(a):
    return pltpu.bitcast(a, jnp.bfloat16)


def _kernel(x_hbm, wq_hbm, wkv_hbm, wo_hbm, o_hbm,
            wq_ref, wkv_ref, wo_ref, ring, xin, k_ref, v_ref, vt_ref, vc_ref,
            s0_ref, max0_ref, s_ref, max_ref, shift_ref, obuf,
            w_sems, head_sems, ring_sems, in_sems, out_sems):
    f32, bf16 = jnp.float32, jnp.bfloat16
    H, C, W = x_hbm.shape
    row_tiles = W // LANES
    row_keys = W // WIN
    key_tiles = (H // WIN) * row_keys // LANES
    groups = key_tiles // N
    rows = BLOCKS * N // row_tiles
    steps = H // rows - 1
    chunks = H // (WIN * CHUNK)
    chunk_rows = WIN * CHUNK
    chunk_keys = CHUNK * row_keys
    tiles = [(u, j) for u in range(BLOCKS) for j in range(N)]

    def tile(t):
        return slice(t * LANES, (t + 1) * LANES)

    def place(u, j):
        return divmod(u * N + j, row_tiles)

    def part(c, n):
        return pl.ds(c * n if isinstance(c, int) else pl.multiple_of(c * n, n), n)

    def dot(a, b):
        return lax.dot(a, b, preferred_element_type=f32)

    def head_copy(w):
        return pltpu.make_async_copy(
            x_hbm.at[pl.ds(w * WIN, WIN)], ring.at[0, pl.ds(w * WIN, WIN)], head_sems.at[w])

    def ring_copy(c, slot):
        return pltpu.make_async_copy(
            x_hbm.at[pl.ds(c * chunk_rows, chunk_rows)], ring.at[slot], ring_sems.at[slot])

    def in_copy(i, slot):
        return pltpu.make_async_copy(x_hbm.at[pl.ds(i * rows, rows)], xin.at[slot], in_sems.at[slot])

    def out_copy(i, slot, off=0, n=rows):
        return pltpu.make_async_copy(
            obuf.at[slot, pl.ds(off, n)], o_hbm.at[pl.ds(i * rows + off, n)], out_sems.at[slot])

    head_copy(0).start()
    w_copies = [pltpu.make_async_copy(src, dst, w_sems.at[n]) for n, (src, dst) in enumerate(
        ((wq_hbm, wq_ref), (wkv_hbm, wkv_ref), (wo_hbm, wo_ref)))]
    for cp in w_copies:
        cp.start()
    head_copy(1).start()
    for cp in w_copies:
        cp.wait()

    win_id = lax.broadcasted_iota(jnp.int32, (LANES // WIN, LANES), 0)
    col_id = lax.broadcasted_iota(jnp.int32, (LANES // WIN, LANES), 1)
    mean_w = jnp.where(col_id // WIN == win_id, 1.0 / (WIN * WIN), 0.0).astype(bf16)
    wkv = wkv_ref[...]
    wk, wv = wkv[:, :C], wkv[:, C:]
    wq_t = wq_ref[...].astype(f32).T.astype(bf16)
    wo_t = wo_ref[...].astype(f32).T.astype(bf16)

    def pool(slot, g):
        w, t = divmod(g, row_tiles)
        cols = _tree_sum(ring[slot, w * WIN + a, :, tile(t)].astype(f32) for a in range(WIN))
        return lax.dot_general(mean_w, cols.astype(bf16), NT, preferred_element_type=f32)

    def fuse_q(k):
        return dot(k.astype(bf16), wq_t) * (C ** -0.5 * LOG2E)

    def project(c, xs, filler):
        xs = jnp.concatenate(xs, axis=0).astype(bf16)
        k = dot(xs, wk)
        v_ref[part(c, chunk_keys), :] = dot(xs, wv).astype(bf16)
        filler()
        k_ref[part(c, chunk_keys // 2), :] = _pack(fuse_q(k))

    def early_scores(c, slot, lo, hi):
        for a in range(lo, hi):
            for t in range(row_tiles):
                s = dot(early_k, ring[slot, a, :, tile(t)])
                s0_ref[c * chunk_rows + a, t] = _fold(s)
                max0_ref[c * chunk_rows + a, t] = _slab_max(s)

    def first_scores(c, k, q, n):
        for u, j in tiles[len(tiles) * q // n:len(tiles) * (q + 1) // n]:
            a, t = place(u, j)
            s = dot(k, xin[1, a, :, tile(t)])
            s_ref[u, j, part(c, chunk_keys // 2), :] = _fold(s)
            max_ref[u, j, c] = _slab_max(s)

    xs = []
    for w in range(CHUNK):
        head_copy(w).wait()
        (head_copy(w + 2) if w + 2 < CHUNK else ring_copy(w + 3 - CHUNK, w + 3 - CHUNK)).start()
        if w * WIN < rows:
            arrived = slice(w * WIN, min(rows, (w + 1) * WIN))
            xin[1, arrived] = ring[0, arrived]
        if w * row_keys == EARLY_KEYS:
            early_scores(0, 0, WIN, 2 * WIN)
        xs += [pool(0, w * row_tiles + t) for t in range(row_tiles)]
        if (w + 1) * row_keys == EARLY_KEYS:
            early_k = fuse_q(dot(jnp.concatenate(xs, axis=0).astype(bf16), wk)).astype(bf16)
            early_scores(0, 0, 0, WIN)
    early_scores(0, 0, 2 * WIN, 2 * WIN + 4)
    project(0, xs, lambda: early_scores(0, 0, 2 * WIN + 4, chunk_rows - 6))
    early_scores(0, 0, chunk_rows - 6, chunk_rows)
    ring_copy(RING, 0).start()

    def stream(c, carry):
        slot = c % RING
        ring_copy(c, slot).wait()
        k = _unpack(k_ref[part(c - 1, chunk_keys // 2), :])
        n = CHUNK * row_tiles
        xs = []
        for g in range(n):
            first_scores(c - 1, k, g, n)
            early_scores(c, slot, 2 * g, 2 * g + 2)
            xs.append(pool(slot, g))
        early_scores(c, slot, 2 * n, chunk_rows - 5)
        project(c, xs, lambda: early_scores(c, slot, chunk_rows - 5, chunk_rows - 2))
        early_scores(c, slot, chunk_rows - 2, chunk_rows)

        @pl.when(c + RING < chunks)
        def _():
            ring_copy(c + RING, slot).start()

    lax.fori_loop(1, chunks, stream, None)
    in_copy(1, 0).start()

    k = _unpack(k_ref[part(chunks - 1, chunk_keys // 2), :])
    for g in range(groups):
        vt = []
        for i in range(N):
            vt.append(lax.dot_general(
                wo_t, v_ref[tile(i * groups + g), :], NT, preferred_element_type=f32))
            vt_ref[i * groups + g] = _pack(vt[i])
            first_scores(chunks - 1, k, g * N + i, (groups + 1) * N)
        if g == groups - 1:
            first_scores(chunks - 1, k, groups, groups + 1)
        lo = [v[C // 2:].astype(bf16).astype(f32) for v in vt]
        mix = [(v[:C // 2] + t * v[C // 2:]).astype(bf16).astype(f32) for v, t in zip(vt, _T)]
        for n, pr in enumerate(_PRODUCTS):
            if pr[0] == 'D':
                val = mix[pr[1]]
            elif pr[0] == 'E':
                val = lo[pr[1]]
            elif pr[0] == 'Z':
                val = mix[pr[1]] - mix[pr[2]]
            elif pr[1] < pr[2]:
                val = (_T[pr[2]] - _T[pr[1]]) * lo[pr[1]] + (mix[pr[1]] - mix[pr[2]])
            else:
                val = (_T[pr[2]] - _T[pr[1]]) * lo[pr[1]] - (mix[pr[2]] - mix[pr[1]])
            vc_ref[g, n] = _pack(val)

    def stored_shift(u, j):
        return _shift([max_ref[u, j, c] for c in range(chunks)])

    for u, j in tiles:
        if (u, j) != LATE:
            shift_ref[u, j] = stored_shift(u, j)

    def probs(h0, u, kt, j, shift):
        r0, r1 = kt * LANES, (kt + 1) * LANES
        a, t = place(u, j)
        s = []
        if r0 < EARLY_KEYS:
            s.append(_unfold(s0_ref[h0 + a, t, r0 // 2:min(r1, EARLY_KEYS) // 2, :]))
        if r1 > EARLY_KEYS:
            s.append(_unfold(s_ref[u, j, max(r0, EARLY_KEYS) // 2:r1 // 2, :]))
        s = jnp.concatenate(s, axis=0) if len(s) > 1 else s[0]
        return jnp.exp2(s.reshape(-1, 8, LANES) - shift[None]).reshape(LANES, LANES)

    def emit(slot, u, j, o, total):
        a, t = place(u, j)
        obuf[slot, a, :, tile(t)] = (o * (1.0 / jnp.sum(total, axis=0, keepdims=True))).astype(bf16)

    jobs = _schedule(groups)

    def step(i, carry):
        slot = i & 1
        in_copy(i + 1, slot).wait()

        @pl.when(i >= 2)
        def _():
            out_copy(i - 2, slot).wait()

        @pl.when(i + 1 < steps)
        def _():
            in_copy(i + 2, 1 - slot).start()

        x_tile, pending, maxes, p_tile, acc, total, cross, seen = {}, {}, {}, {}, {}, {}, {}, {}
        late_shift = stored_shift(*LATE)

        def store_scores():
            for u, j, r in list(pending):
                if (u, r // LANES, j) in p_tile and (u, (r + UNIT - 1) // LANES, j) in p_tile:
                    s_ref[u, j, r // 2:(r + UNIT) // 2, :] = pending.pop((u, j, r))

        def prob(u, kt, j):
            if (u, kt, j) not in p_tile:
                shift = late_shift if (u, j) == LATE else shift_ref[u, j]
                p_tile[u, kt, j] = probs(i * rows, u, kt, j, shift)
                store_scores()
            return p_tile[u, kt, j]

        def score(u, j, r):
            if (u, j) not in x_tile:
                a, t = place(u, j)
                x_tile[u, j] = xin[slot, a, :, tile(t)]
            s = dot(_unpack(k_ref[r // 2:(r + UNIT) // 2, :]), x_tile[u, j])
            pending[u, j, r] = _fold(s)
            store_scores()
            m, c = maxes.setdefault((u, j), {}), r // chunk_keys
            m[c] = jnp.maximum(m[c], _slab_max(s)) if c in m else _slab_max(s)

        def finish(u, j):
            upper, lower = acc[u, ('D', j)], acc[u, ('E', j)]
            for other in range(N):
                if other == j:
                    continue
                a, b = sorted((other, j))
                if (u, a, b) not in cross:
                    w = acc[u, ('X', a, b)] + acc[u, ('X', b, a)] + acc[u, ('Z', a, b)]
                    cross[u, a, b] = w if _T[b] - _T[a] == 1 else w * (1.0 / (_T[b] - _T[a]))
                upper = upper + acc[u, ('X', other, j)]
                lower = lower + cross[u, a, b] if j == b else lower - cross[u, a, b]
            emit(slot, u, j, jnp.concatenate([upper - _T[j] * lower, lower], axis=0), total[u, j])

        def value(u, g, pr):
            p = [prob(u, kt * groups + g, j) for kt, j in _cells(pr)]
            p = p[0] - p[1] if pr[0] == 'Z' else _tree_sum(p)
            if pr[0] == 'D':
                total[u, pr[1]] = _slab_sum(p) + total[u, pr[1]] if g else _slab_sum(p)
            o = dot(_unpack(vc_ref[g, _PRODUCTS.index(pr)]), p)
            acc[u, pr] = o + acc[u, pr] if g else o
            for j in sorted(pr[1:]):
                seen[u, j] = seen.get((u, j), 0) + 1
                if seen[u, j] == (3 * N - 1) * groups:
                    finish(u, j)

        for kind, *args in jobs:
            (score if kind == 'score' else value)(*args)
        assert not pending

        for (u, j), m in maxes.items():
            a, t = place(u, j)
            m[0] = jnp.maximum(m[0], max0_ref[(i + 1) * rows + a, t])
            if (u, j) == LATE:
                for c, v in m.items():
                    max_ref[u, j, c] = v
            else:
                shift_ref[u, j] = _shift(list(m.values()))
        out_copy(i, slot).start()

    lax.fori_loop(0, steps, step, None)

    slot = steps % 2
    out_copy(steps - 2, slot).wait()
    shift_ref[LATE] = stored_shift(*LATE)
    for u, j in tiles:
        for kt in range(key_tiles):
            p = probs(steps * rows, u, kt, j, shift_ref[u, j])
            o_part, total_part = dot(_unpack(vt_ref[kt]), p), _slab_sum(p)
            o, total = (o + o_part, total + total_part) if kt else (o_part, total_part)
        emit(slot, u, j, o, total)
        a, t = place(u, j)
        if t == row_tiles - 1:
            out_copy(steps, slot, a, 1).start()
    out_copy(steps - 1, 1 - slot).wait()
    for a in range(rows):
        out_copy(steps, slot, a, 1).wait()


@jax.jit
def pallas_standalone__window_attn_twins__vision_kernel(
    x: jax.Array,
    wq: jax.Array,
    wkv: jax.Array,
    wo: jax.Array,
):
    B, H, W, C = x.shape
    assert (B, H, W, C) == (1, 384, 384, 2 * UNIT)
    f32, bf16, u32 = jnp.float32, jnp.bfloat16, jnp.uint32
    keys = (H // WIN) * (W // WIN)
    rows = BLOCKS * N // (W // LANES)
    out = pl.pallas_call(
        _kernel,
        out_shape=jax.ShapeDtypeStruct((H, C, W), x.dtype),
        in_specs=[pl.BlockSpec(memory_space=pl.ANY)] * 4,
        out_specs=pl.BlockSpec(memory_space=pl.ANY),
        scratch_shapes=[
            pltpu.VMEM(wq.shape, bf16),
            pltpu.VMEM(wkv.shape, bf16),
            pltpu.VMEM(wo.shape, bf16),
            pltpu.VMEM((RING, CHUNK * WIN, C, W), bf16),
            pltpu.VMEM((2, rows, C, W), bf16),
            pltpu.VMEM((keys // 2, C), u32),
            pltpu.VMEM((keys, C), bf16),
            pltpu.VMEM((keys // LANES, C // 2, LANES), u32),
            pltpu.VMEM((keys // (LANES * N), len(_PRODUCTS), C // 4, LANES), u32),
            pltpu.VMEM((H, W // LANES, EARLY_KEYS // 2, 2 * LANES), bf16),
            pltpu.VMEM((H, W // LANES, 8, LANES), f32),
            pltpu.VMEM((BLOCKS, N, keys // 2, 2 * LANES), bf16),
            pltpu.VMEM((BLOCKS, N, H // (WIN * CHUNK), 8, LANES), f32),
            pltpu.VMEM((BLOCKS, N, 8, LANES), f32),
            pltpu.VMEM((2, rows, C, W), bf16),
            pltpu.SemaphoreType.DMA((3,)),
            pltpu.SemaphoreType.DMA((CHUNK,)),
            pltpu.SemaphoreType.DMA((RING,)),
            pltpu.SemaphoreType.DMA((2,)),
            pltpu.SemaphoreType.DMA((2,)),
        ],
        compiler_params=pltpu.CompilerParams(
            vmem_limit_bytes=110 * 1024 * 1024, disable_bounds_checks=True),
    )(jnp.transpose(x, (0, 1, 3, 2)).reshape(H, C, W), wq, wkv, wo)
    return jnp.transpose(out.reshape(B, H, C, W), (0, 1, 3, 2))
```

```python
import functools

import jax
import jax.numpy as jnp
from jax import lax
import jax.experimental.pallas as pl
import jax.experimental.pallas.tpu as pltpu

WIN = 8
LANES = 128
UNIT = 48
N = 6
BLOCKS = 6
EARLY_KEYS = 144
CHUNK = 4
LEAD, TAIL = 2, 2
LATE = (0, 1)
LOG2E = 1.4426950408889634
NT = (((1,), (1,)), ((), ()))

_T = (-1.25, -0.75, -0.25, 0.25, 0.75, 1.25)
_PRODUCTS = [('D', j) for j in range(N)] + [('E', j) for j in range(N)] + [
    pr for i in range(N) for j in range(i + 1, N) for pr in (('X', i, j), ('X', j, i), ('Z', i, j))]

_ORDER = (
    'X10|X01 Z01|X02 X30|X20 Z02|X03 Z03|X40 X05|X04 Z04|X50 Z05,E0,D0 X31|X21|X13 Z13|'
    'X12 Z12|X14 X15,X41 Z14|E1,X51 Z15,D1|X23,X24 X25|X32 Z23|X42 Z24|E2,Z25 X52,D2,X34 X35|'
    'X43 Z34|X53 Z35,E3,D3|X45|Z45 X54,E4,D4,E5,D5',
    'X10|X01 Z01|X02 X30|X20 Z02|X03 Z03|X40 X05|X04 Z04|E0,X50 Z05,D0 X13|X12|X21 Z12|'
    'X31 Z13|X14 X15,X41 Z14|Z15 X51,E1,D1|X23,X32 Z23|X42 X25|X24 Z24|E2,Z25 X52,D2|X34 X35|'
    'X53 Z35|X43 Z34|E3,D3|X45|E4,X54 Z45,D4,D5,E5',
    'X10|X01 Z01|X02 X30,X20 Z02,X03 Z03|X40 X05|X04 Z04|E0,X50 Z05,D0 X13|X21|X31 Z13|'
    'X14 X15|X12 Z12,X41 Z14|E1,X51 Z15,D1|X32,X23 Z23|X24 X25|X42 Z24|Z25 X52,E2,D2|'
    'X34 X35,X43 Z34|X53 Z35,E3,D3|X45|E4,X54 Z45,D4,D5,E5',
    'X01|X10 Z01|X02 X03,X20 Z02|X30 Z03|X40 X05|X04 Z04|E0,X50 Z05,D0 X13|X21|Z12 X12|'
    'X31 Z13|X14 X15,X41 Z14|E1,X51 Z15,D1|X23,X32 Z23|X24 X25|X42 Z24|E2,Z25 X52,D2|X34 X35|'
    'Z34 X43|X53 Z35,D3,E3|X45|E4,X54 Z45,D4,E5,D5',
    'X10|X01 Z01|X02 X03|X20 Z02|X30 Z03|X40 X05|Z04 X04|E0,X50 Z05,D0 X31|X21|Z12 X12|'
    'X14 X15|X13 Z13,X41 Z14|E1,X51 Z15,D1|X23,X32 Z23|X24 X25|X42 Z24|E2,Z25 X52,D2|X35 X34|'
    'X43 Z34|X53 Z35,E3,D3|X45|X54 Z45|E4,D4,D5,E5',
    'X10|X01 Z01|X02 X03|X20 Z02|X30 Z03|X40 X05|X04 Z04|E0,Z05 X50,D0 X13,X21|Z12 X12|'
    'X31 Z13|X14 X15,X41 Z14|E1,X51 Z15,D1|X23,X32 Z23|X24 X25|X42 Z24|E2,Z25 X52,D2|X34 X35|'
    'Z34 X43|X53 Z35,E3,D3|X45|E4,X54 Z45,D4,E5,D5',
)
_SPARE = (23, 26)


def _cells(pr):
    if pr[0] == 'D':
        return [(i, pr[1]) for i in range(N)]
    if pr[0] == 'E':
        return [(pr[1], j) for j in range(N)]
    if pr[0] == 'X':
        return [(pr[1], pr[2])]
    return [(pr[2], pr[1]), (pr[1], pr[2])]


def _schedule(groups):
    work = [[(u, g, (k[0],) + tuple(map(int, k[1:]))) for k in rnd.split()]
            for u in range(BLOCKS) for phase in _ORDER[u % len(_ORDER)].split('|')
            for g in range(groups) for rnd in phase.split(',')]
    scores = [(u, j, r) for u in range(BLOCKS) for j in range(N)
              for r in range(EARLY_KEYS, N * groups * LANES, UNIT)]
    n_spare = (len(scores) - sum(4 - len(w) for w in work)) // 4 - LEAD - TAIL
    per_block = len(work) // BLOCKS
    spare = [u * per_block + e for e in _SPARE for u in range(BLOCKS)][:n_spare]
    rounds = [[]] * LEAD
    for n, w in enumerate(work):
        rounds = rounds + [w] + [[]] * spare.count(n)
    rounds = rounds + [[]] * (n_spare - len(spare) + TAIL)

    first = {}
    for n, rnd in enumerate(rounds):
        for u, g, pr in rnd:
            for i, j in _cells(pr):
                first.setdefault((u, i * groups + g, j), n)

    def free(u, j, r):
        return max(first[u, r // LANES, j], first[u, (r + UNIT - 1) // LANES, j])

    span = groups * LANES
    last = [s for s in scores if s[:2] == LATE][-4 * TAIL:]
    todo = sorted((s for s in scores if s not in last),
                  key=lambda s: (free(s[0], s[1], s[2] // span * span), s))
    jobs = []
    for n, rnd in enumerate(rounds):
        jobs += [('value',) + w for w in rnd]
        for _ in range(4 - len(rnd)):
            if not todo:
                todo, last = last, []
            s = next((s for s in todo if free(*s) <= n), todo[-1])
            todo.remove(s)
            jobs.append(('score',) + s)
    return jobs + [('score',) + s for s in todo + last]


def _tree_sum(xs):
    xs = list(xs)
    while len(xs) > 1:
        xs = [xs[i] + xs[i + 1] if i + 1 < len(xs) else xs[i] for i in range(0, len(xs), 2)]
    return xs[0]


def _fold(s):
    s = s.reshape(-1, 16, LANES)
    return jnp.concatenate([s[:, :8], s[:, 8:]], axis=2).reshape(-1, 2 * LANES).astype(jnp.bfloat16)


def _unfold(b):
    b = b.astype(jnp.float32).reshape(-1, 1, 8, 2 * LANES)
    return jnp.concatenate([b[..., :LANES], b[..., LANES:]], axis=1).reshape(-1, 8, LANES)


def _slab_max(s):
    return jnp.max(s.reshape(-1, 8, LANES), axis=0)


def _slab_sum(s):
    return jnp.sum(s.reshape(-1, 8, LANES), axis=0)


def _shift(maxes):
    m = functools.reduce(jnp.maximum, maxes)
    m = jnp.broadcast_to(jnp.max(m, axis=0, keepdims=True), m.shape)
    norm = jnp.log2(jnp.sum(_tree_sum(jnp.exp2(v - m) for v in maxes), axis=0, keepdims=True))
    return m.astype(jnp.bfloat16).astype(jnp.float32) + norm


def _pack(a):
    return pltpu.bitcast(a.astype(jnp.bfloat16), jnp.uint32)


def _unpack(a):
    return pltpu.bitcast(a, jnp.bfloat16)


def _kernel(x_hbm, wq_hbm, wkv_hbm, wo_hbm, o_hbm,
            wq_ref, wkv_ref, wo_ref, ring, xin, k_ref, xs_ref, vt_ref, vc_ref,
            s0_ref, max0_ref, s_ref, max_ref, shift_ref, obuf,
            w_sems, head_sems, ring_sems, in_sems, out_sems):
    f32, bf16 = jnp.float32, jnp.bfloat16
    H, C, W = x_hbm.shape
    row_tiles = W // LANES
    row_keys = W // WIN
    key_tiles = (H // WIN) * row_keys // LANES
    groups = key_tiles // N
    rows = BLOCKS * N // row_tiles
    steps = H // rows - 1
    chunks = H // (WIN * CHUNK)
    chunk_rows = WIN * CHUNK
    chunk_keys = CHUNK * row_keys
    tiles = [(u, j) for u in range(BLOCKS) for j in range(N)]

    def tile(t):
        return slice(t * LANES, (t + 1) * LANES)

    def place(u, j):
        return divmod(u * N + j, row_tiles)

    def part(c, n):
        return pl.ds(c * n if isinstance(c, int) else pl.multiple_of(c * n, n), n)

    def dot(a, b):
        return lax.dot(a, b, preferred_element_type=f32)

    def head_copy(w):
        return pltpu.make_async_copy(
            x_hbm.at[pl.ds(w * WIN, WIN)], ring.at[0, pl.ds(w * WIN, WIN)], head_sems.at[w])

    def ring_copy(c, slot):
        return pltpu.make_async_copy(
            x_hbm.at[pl.ds(c * chunk_rows, chunk_rows)], ring.at[slot], ring_sems.at[slot])

    def in_copy(i, slot):
        return pltpu.make_async_copy(x_hbm.at[pl.ds(i * rows, rows)], xin.at[slot], in_sems.at[slot])

    def out_copy(i, slot, off=0, n=rows):
        return pltpu.make_async_copy(
            obuf.at[slot, pl.ds(off, n)], o_hbm.at[pl.ds(i * rows + off, n)], out_sems.at[slot])

    head_copy(0).start()
    w_copies = [pltpu.make_async_copy(src, dst, w_sems.at[n]) for n, (src, dst) in enumerate(
        ((wq_hbm, wq_ref), (wkv_hbm, wkv_ref), (wo_hbm, wo_ref)))]
    for cp in w_copies:
        cp.start()
    head_copy(1).start()
    for cp in w_copies:
        cp.wait()

    win_id = lax.broadcasted_iota(jnp.int32, (LANES // WIN, LANES), 0)
    col_id = lax.broadcasted_iota(jnp.int32, (LANES // WIN, LANES), 1)
    mean_w = jnp.where(col_id // WIN == win_id, 1.0 / (WIN * WIN), 0.0).astype(bf16)
    wkv = wkv_ref[...]
    wk = wkv[:, :C]
    wq_t = wq_ref[...].astype(f32).T.astype(bf16)
    wvo_t = dot(wkv[:, C:], wo_ref[...]).T.astype(bf16)

    def pool(slot, g):
        w, t = divmod(g, row_tiles)
        cols = _tree_sum(ring[slot, w * WIN + a, :, tile(t)].astype(f32) for a in range(WIN))
        return lax.dot_general(mean_w, cols.astype(bf16), NT, preferred_element_type=f32)

    def fuse_q(k):
        return dot(k.astype(bf16), wq_t) * (C ** -0.5 * LOG2E)

    def project(c, xs, filler):
        xs = jnp.concatenate(xs, axis=0).astype(bf16)
        k = dot(xs, wk)
        xs_ref[part(c, chunk_keys), :] = xs
        filler()
        k_ref[part(c, chunk_keys // 2), :] = _pack(fuse_q(k))

    def early_scores(c, slot, lo, hi):
        for a in range(lo, hi):
            for t in range(row_tiles):
                s = dot(early_k, ring[slot, a, :, tile(t)])
                s0_ref[c * chunk_rows + a, t] = _fold(s)
                max0_ref[c * chunk_rows + a, t] = _slab_max(s)

    def first_scores(c, k, q, n):
        for u, j in tiles[len(tiles) * q // n:len(tiles) * (q + 1) // n]:
            a, t = place(u, j)
            s = dot(k, xin[1, a, :, tile(t)])
            s_ref[u, j, part(c, chunk_keys // 2), :] = _fold(s)
            max_ref[u, j, c] = _slab_max(s)

    xs = []
    for w in range(CHUNK):
        head_copy(w).wait()
        if w + 2 < CHUNK:
            head_copy(w + 2).start()
        elif w + 2 == CHUNK:
            ring_copy(1, 1).start()
        if w * WIN < rows:
            arrived = slice(w * WIN, min(rows, (w + 1) * WIN))
            xin[1, arrived] = ring[0, arrived]
        if w * row_keys == EARLY_KEYS:
            early_scores(0, 0, WIN, 2 * WIN)
        xs += [pool(0, w * row_tiles + t) for t in range(row_tiles)]
        if (w + 1) * row_keys == EARLY_KEYS:
            early_k = fuse_q(dot(jnp.concatenate(xs, axis=0).astype(bf16), wk)).astype(bf16)
            early_scores(0, 0, 0, WIN)
    early_scores(0, 0, 2 * WIN, 2 * WIN + 4)
    project(0, xs, lambda: early_scores(0, 0, 2 * WIN + 4, chunk_rows - 6))
    early_scores(0, 0, chunk_rows - 6, chunk_rows)

    def stream(c, carry):
        slot = c & 1
        ring_copy(c, slot).wait()

        @pl.when(c + 1 < chunks)
        def _():
            ring_copy(c + 1, 1 - slot).start()

        k = _unpack(k_ref[part(c - 1, chunk_keys // 2), :])
        n = CHUNK * row_tiles
        xs = []
        for g in range(n):
            first_scores(c - 1, k, g, n)
            early_scores(c, slot, 2 * g, 2 * g + 2)
            xs.append(pool(slot, g))
        early_scores(c, slot, 2 * n, chunk_rows - 5)
        project(c, xs, lambda: early_scores(c, slot, chunk_rows - 5, chunk_rows - 2))
        early_scores(c, slot, chunk_rows - 2, chunk_rows)

    lax.fori_loop(1, chunks, stream, None)
    in_copy(1, 0).start()

    k = _unpack(k_ref[part(chunks - 1, chunk_keys // 2), :])
    for g in range(groups):
        vt = []
        for i in range(N):
            vt.append(lax.dot_general(
                wvo_t, xs_ref[tile(i * groups + g), :], NT, preferred_element_type=f32))
            vt_ref[i * groups + g] = _pack(vt[i])
            first_scores(chunks - 1, k, g * N + i, (groups + 1) * N)
        if g == groups - 1:
            first_scores(chunks - 1, k, groups, groups + 1)
        lo = [v[C // 2:].astype(bf16).astype(f32) for v in vt]
        mix = [(v[:C // 2] + t * v[C // 2:]).astype(bf16).astype(f32) for v, t in zip(vt, _T)]
        for n, pr in enumerate(_PRODUCTS):
            if pr[0] == 'D':
                val = mix[pr[1]]
            elif pr[0] == 'E':
                val = lo[pr[1]]
            elif pr[0] == 'Z':
                val = mix[pr[1]] - mix[pr[2]]
            elif pr[1] < pr[2]:
                val = (_T[pr[2]] - _T[pr[1]]) * lo[pr[1]] + (mix[pr[1]] - mix[pr[2]])
            else:
                val = (_T[pr[2]] - _T[pr[1]]) * lo[pr[1]] - (mix[pr[2]] - mix[pr[1]])
            vc_ref[g, n] = _pack(val)

    def stored_shift(u, j):
        return _shift([max_ref[u, j, c] for c in range(chunks)])

    for u, j in tiles:
        if (u, j) != LATE:
            shift_ref[u, j] = stored_shift(u, j)

    def probs(h0, u, kt, j, shift):
        r0, r1 = kt * LANES, (kt + 1) * LANES
        a, t = place(u, j)
        s = []
        if r0 < EARLY_KEYS:
            s.append(_unfold(s0_ref[h0 + a, t, r0 // 2:min(r1, EARLY_KEYS) // 2, :]))
        if r1 > EARLY_KEYS:
            s.append(_unfold(s_ref[u, j, max(r0, EARLY_KEYS) // 2:r1 // 2, :]))
        s = jnp.concatenate(s, axis=0) if len(s) > 1 else s[0]
        return jnp.exp2(s - shift[None]).reshape(LANES, LANES)

    def run(i, slot, jobs, row_done=None):
        x_tile, pending, maxes, p_tile, acc, total, cross, seen = {}, {}, {}, {}, {}, {}, {}, {}
        late_shift = stored_shift(*LATE)
        vt_tile = functools.cache(lambda kt: _unpack(vt_ref[kt]))

        def store_scores():
            for u, j, r in list(pending):
                if (u, r // LANES, j) in p_tile and (u, (r + UNIT - 1) // LANES, j) in p_tile:
                    s_ref[u, j, r // 2:(r + UNIT) // 2, :] = pending.pop((u, j, r))

        def prob(u, kt, j):
            if (u, kt, j) not in p_tile:
                shift = late_shift if (u, j) == LATE else shift_ref[u, j]
                p_tile[u, kt, j] = probs(i * rows, u, kt, j, shift)
                store_scores()
            return p_tile[u, kt, j]

        def score(u, j, r):
            if (u, j) not in x_tile:
                a, t = place(u, j)
                x_tile[u, j] = xin[slot, a, :, tile(t)]
            s = dot(_unpack(k_ref[r // 2:(r + UNIT) // 2, :]), x_tile[u, j])
            pending[u, j, r] = _fold(s)
            store_scores()
            m, c = maxes.setdefault((u, j), {}), r // chunk_keys
            m[c] = jnp.maximum(m[c], _slab_max(s)) if c in m else _slab_max(s)

        def emit(u, j, o):
            a, t = place(u, j)
            o = o * (1.0 / jnp.sum(total[u, j], axis=0, keepdims=True))
            obuf[slot, a, :, tile(t)] = o.astype(bf16)
            seen[a] = seen.get(a, 0) + 1
            if row_done and seen[a] == row_tiles:
                row_done(a)

        def plain(u, j, kt):
            p = prob(u, kt, j)
            o = dot(vt_tile(kt), p)
            acc[u, j], total[u, j] = (acc[u, j] + o, total[u, j] + _slab_sum(p)) if kt else (o, _slab_sum(p))
            if kt == key_tiles - 1:
                emit(u, j, acc[u, j])

        def finish(u, j):
            upper, lower = acc[u, ('D', j)], acc[u, ('E', j)]
            for other in range(N):
                if other == j:
                    continue
                a, b = sorted((other, j))
                if (u, a, b) not in cross:
                    w = acc[u, ('X', a, b)] + acc[u, ('X', b, a)] + acc[u, ('Z', a, b)]
                    cross[u, a, b] = w if _T[b] - _T[a] == 1 else w * (1.0 / (_T[b] - _T[a]))
                upper = upper + acc[u, ('X', other, j)]
                lower = lower + cross[u, a, b] if j == b else lower - cross[u, a, b]
            emit(u, j, jnp.concatenate([upper - _T[j] * lower, lower], axis=0))

        def value(u, g, pr):
            p = [prob(u, kt * groups + g, j) for kt, j in _cells(pr)]
            p = p[0] - p[1] if pr[0] == 'Z' else _tree_sum(p)
            if pr[0] == 'D':
                total[u, pr[1]] = _slab_sum(p) + total[u, pr[1]] if g else _slab_sum(p)
            o = dot(_unpack(vc_ref[g, _PRODUCTS.index(pr)]), p)
            acc[u, pr] = o + acc[u, pr] if g else o
            for j in sorted(pr[1:]):
                seen[u, j] = seen.get((u, j), 0) + 1
                if seen[u, j] == (3 * N - 1) * groups:
                    finish(u, j)

        for kind, *args in jobs:
            dict(score=score, value=value, plain=plain)[kind](*args)
        assert not pending

        for (u, j), m in maxes.items():
            a, t = place(u, j)
            m[0] = jnp.maximum(m[0], max0_ref[(i + 1) * rows + a, t])
            if (u, j) == LATE:
                for c, v in m.items():
                    max_ref[u, j, c] = v
            else:
                shift_ref[u, j] = _shift(list(m.values()))

    jobs = _schedule(groups)

    def step(i, carry):
        slot = i & 1
        in_copy(i + 1, slot).wait()

        @pl.when(i >= 2)
        def _():
            out_copy(i - 2, slot).wait()

        @pl.when(i + 1 < steps)
        def _():
            in_copy(i + 2, 1 - slot).start()

        run(i, slot, jobs)
        out_copy(i, slot).start()

    lax.fori_loop(0, steps, step, None)

    slot = steps % 2
    out_copy(steps - 2, slot).wait()
    run(steps, slot, [('plain', u, j, kt) for u, j in tiles for kt in range(key_tiles)],
        lambda a: out_copy(steps, slot, a, 1).start())
    out_copy(steps - 1, 1 - slot).wait()
    for a in range(rows):
        out_copy(steps, slot, a, 1).wait()


@jax.jit
def pallas_standalone__window_attn_twins__vision_kernel(
    x: jax.Array,
    wq: jax.Array,
    wkv: jax.Array,
    wo: jax.Array,
):
    B, H, W, C = x.shape
    assert (B, H, W, C) == (1, 384, 384, 2 * UNIT)
    f32, bf16, u32 = jnp.float32, jnp.bfloat16, jnp.uint32
    keys = (H // WIN) * (W // WIN)
    rows = BLOCKS * N // (W // LANES)
    out = pl.pallas_call(
        _kernel,
        out_shape=jax.ShapeDtypeStruct((H, C, W), x.dtype),
        in_specs=[pl.BlockSpec(memory_space=pl.ANY)] * 4,
        out_specs=pl.BlockSpec(memory_space=pl.ANY),
        scratch_shapes=[
            pltpu.VMEM(wq.shape, bf16),
            pltpu.VMEM(wkv.shape, bf16),
            pltpu.VMEM(wo.shape, bf16),
            pltpu.VMEM((2, CHUNK * WIN, C, W), bf16),
            pltpu.VMEM((2, rows, C, W), bf16),
            pltpu.VMEM((keys // 2, C), u32),
            pltpu.VMEM((keys, C), bf16),
            pltpu.VMEM((keys // LANES, C // 2, LANES), u32),
            pltpu.VMEM((keys // (LANES * N), len(_PRODUCTS), C // 4, LANES), u32),
            pltpu.VMEM((H, W // LANES, EARLY_KEYS // 2, 2 * LANES), bf16),
            pltpu.VMEM((H, W // LANES, 8, LANES), f32),
            pltpu.VMEM((BLOCKS, N, keys // 2, 2 * LANES), bf16),
            pltpu.VMEM((BLOCKS, N, H // (WIN * CHUNK), 8, LANES), f32),
            pltpu.VMEM((BLOCKS, N, 8, LANES), f32),
            pltpu.VMEM((2, rows, C, W), bf16),
            pltpu.SemaphoreType.DMA((3,)),
            pltpu.SemaphoreType.DMA((CHUNK,)),
            pltpu.SemaphoreType.DMA((2,)),
            pltpu.SemaphoreType.DMA((2,)),
            pltpu.SemaphoreType.DMA((2,)),
        ],
        compiler_params=pltpu.CompilerParams(
            vmem_limit_bytes=110 * 1024 * 1024, disable_bounds_checks=True),
    )(jnp.transpose(x, (0, 1, 3, 2)).reshape(H, C, W), wq, wkv, wo)
    return jnp.transpose(out.reshape(B, H, C, W), (0, 1, 3, 2))
```
